```python
import jax
import jax.numpy as jnp

def _softmax(x, axis=-1):
    return jax.nn.softmax(x, axis=axis)

def _gelu(x):
    return jax.nn.gelu(x, approximate=True)

def _silu(x):
    return jax.nn.silu(x)

def _sigmoid(x):
    return jax.nn.sigmoid(x)

def _layernorm(x, axis=-1, eps=1e-05):
    m = jnp.mean(x, axis=axis, keepdims=True)
    v = jnp.var(x, axis=axis, keepdims=True)
    return (x - m) / jnp.sqrt(v + eps)

def _scatter_add(tgt, idx, src, axis=0):
    return tgt.at[idx].add(src)

def _segment_sum(src, seg, n):
    return jax.ops.segment_sum(src, seg, n)

class _Rng:

    def __init__(self, key):
        self._k = key

    def _next(self):
        self._k, sub = jax.random.split(self._k)
        return sub

    def normal(self, shape):
        return jax.random.normal(self._next(), shape, dtype=jnp.bfloat16)

    def randint(self, lo, hi, shape):
        return jax.random.randint(self._next(), shape, lo, hi, dtype=jnp.int32)

    def uniform(self, shape, lo=0.0, hi=1.0):
        return jax.random.uniform(self._next(), shape, jnp.bfloat16, lo, hi)

    def permutation(self, n):
        return jax.random.permutation(self._next(), n)
kernel_name = 'standalone__dilated_atrous__vision'

def setup_inputs():
    _rng = _Rng(jax.random.key(int.from_bytes(__import__("os").urandom(4), "little")))
    _w = lambda a: (lambda t: t.astype(jnp.bfloat16) if jnp.issubdtype(t.dtype, jnp.floating) else t)(jnp.asarray(a))
    H = W = 384
    C = 384
    k = 1
    return {'x': _w((lambda *s: _rng.normal(s) * 0.05)(1, H, W, C)), 'w': _w((lambda *s: _rng.normal(s) * 0.05)(k, k, C, C) * (1.0 / (k * C ** 0.5)))}

def reference(x, w):
    B, H, W, C = x.shape
    k = 1
    rate = 2
    pad = (k - 1) * rate // 2
    xp = jnp.pad(x, ((0, 0), (pad, pad), (pad, pad), (0, 0)))
    out = jnp.zeros_like(x)
    for i in range(k):
        for j in range(k):
            tap = xp[:, i * rate:i * rate + H, j * rate:j * rate + W, :].copy()
            out = out + jnp.einsum('bhwc,co->bhwo', tap, w[i, j])
    return out
```

```python
import jax
import jax.numpy as jnp
import jax.experimental.pallas as pl
import jax.experimental.pallas.tpu as pltpu


@jax.jit
def pallas_standalone__dilated_atrous__vision_kernel(
    x: jax.Array,
    w: jax.Array,
):
    B, H, W, C = x.shape
    Co = w.shape[-1]
    M = B * H * W
    x2 = x.reshape(M, C)
    w2 = w.reshape(C, Co)
    tm = 2048

    def kernel_function(x_ref, w_ref, o_ref):
        o_ref[...] = jnp.dot(
            x_ref[...], w_ref[...], preferred_element_type=jnp.float32
        ).astype(o_ref.dtype)

    out = pl.pallas_call(
        kernel_function,
        grid=(M // tm,),
        in_specs=[
            pl.BlockSpec((tm, C), lambda i: (i, 0)),
            pl.BlockSpec((C, Co), lambda i: (0, 0)),
        ],
        out_specs=pl.BlockSpec((tm, Co), lambda i: (i, 0)),
        out_shape=jax.ShapeDtypeStruct((M, Co), x.dtype),
        compiler_params=pltpu.CompilerParams(
            dimension_semantics=("arbitrary",),
            vmem_limit_bytes=64 * 1024 * 1024,
        ),
    )(x2, w2)
    return out.reshape(B, H, W, Co)
```

```python
import jax
import jax.numpy as jnp
import jax.experimental.pallas as pl
import jax.experimental.pallas.tpu as pltpu

_S = 8
_RB = 128
_R = 32
_NI = 60
_NO = 84
_U0 = 48
_UPS = 6


@jax.jit
def pallas_standalone__dilated_atrous__vision_kernel(
    x: jax.Array,
    w: jax.Array,
):
    B, H, W, C = x.shape
    Co = w.shape[-1]
    M = B * H * W
    S, rb, r, NI, NO, U0, UPS = _S, _RB, _R, _NI, _NO, _U0, _UPS
    JS = NO
    R = M // S
    n = R // rb
    nw = rb // r
    nu = n * nw
    assert M == S * n * rb and JS + NI >= n and NI <= n and NO <= n
    uend = U0 + (n - JS) * UPS
    assert uend <= nu
    for j in range(JS, n):
        assert (U0 + (j - JS + 1) * UPS - 1) // nw <= j
        assert (j - NO + 1) * nw <= U0 + (j - JS) * UPS

    def kernel_function(x_hbm, w_hbm, o_hbm, ibuf, obuf, wbuf, rsem, wsem, ksem):
        def rd(j, slot):
            return pltpu.make_async_copy(
                x_hbm.at[:, pl.ds(pl.multiple_of(j * rb, rb), rb)],
                ibuf.at[slot], rsem.at[slot])

        def wr_start(u):
            slot = (u // nw) % NO
            pltpu.make_async_copy(
                obuf.at[slot, u % nw],
                o_hbm.at[:, pl.ds(pl.multiple_of(u * r, r), r)],
                wsem.at[slot]).start()

        def wr_wait(slot):
            pltpu.make_async_copy(obuf.at[slot], obuf.at[slot], wsem.at[slot]).wait()

        def compute(islot, oslot):
            xv = ibuf[islot].reshape(S * rb, C)
            y = jnp.dot(xv, wbuf[...], preferred_element_type=jnp.float32)
            y = y.astype(obuf.dtype).reshape(S, rb, Co)
            for q in range(nw):
                obuf[oslot, q] = y[:, q * r:(q + 1) * r, :]

        wcp = pltpu.make_async_copy(w_hbm, wbuf, ksem)
        wcp.start()

        def fill(j, c):
            rd(j, j).start()
            return c
        jax.lax.fori_loop(0, NI, fill, 0)
        wcp.wait()

        def phase1(j, c):
            s = j % NI
            rd(j, s).wait()
            compute(s, j)

            @pl.when(j + NI < n)
            def _():
                rd(j + NI, s).start()
            return c
        jax.lax.fori_loop(0, JS, phase1, 0)

        def drain(j, c):
            rd(j, j % NI).wait()
            return c
        jax.lax.fori_loop(JS, n - 1, drain, 0)

        def issue(u, c):
            wr_start(u)
            return c
        jax.lax.fori_loop(0, U0, issue, 0)
        rd(n - 1, (n - 1) % NI).wait()

        def phase2(j, c):
            os_ = j - NO
            wr_wait(os_)
            compute(j % NI, os_)
            u0 = U0 + (j - JS) * UPS
            for q in range(UPS):
                wr_start(u0 + q)
            return c
        jax.lax.fori_loop(JS, n, phase2, 0)

        jax.lax.fori_loop(uend, nu, issue, 0)

        def final_wait(j, c):
            wr_wait(j % NO)
            return c
        jax.lax.fori_loop(n - NO, n, final_wait, 0)

    assert n - NO <= NO
    out = pl.pallas_call(
        kernel_function,
        in_specs=[pl.BlockSpec(memory_space=pl.ANY), pl.BlockSpec(memory_space=pl.ANY)],
        out_specs=pl.BlockSpec(memory_space=pl.ANY),
        out_shape=jax.ShapeDtypeStruct((S, R, Co), x.dtype),
        scratch_shapes=[
            pltpu.VMEM((NI, S, rb, C), x.dtype),
            pltpu.VMEM((NO, nw, S, r, Co), x.dtype),
            pltpu.VMEM((C, Co), w.dtype),
            pltpu.SemaphoreType.DMA((NI,)),
            pltpu.SemaphoreType.DMA((NO,)),
            pltpu.SemaphoreType.DMA(()),
        ],
        compiler_params=pltpu.CompilerParams(
            vmem_limit_bytes=120 * 1024 * 1024,
            disable_bounds_checks=True,
            disable_semaphore_checks=True,
        ),
    )(x.reshape(S, R, C), w.reshape(C, Co))
    return out.reshape(B, H, W, Co)
```

```python
import jax
import jax.numpy as jnp
import jax.experimental.pallas as pl
import jax.experimental.pallas.tpu as pltpu

_S = 6
_S1 = 5
_RB = 192
_RR = 32
_RW = 48
_NI = 56
_JS = 73
_LAG = 26
_PF = 24
_PPS = 10
_U0 = 64
_UPS = 6


@jax.jit
def pallas_standalone__dilated_atrous__vision_kernel(
    x: jax.Array,
    w: jax.Array,
):
    B, H, W, C = x.shape
    Co = w.shape[-1]
    M = B * H * W
    S, S1, rb, rr, rw = _S, _S1, _RB, _RR, _RW
    NI, JS, LAG, PF, PPS, U0, UPS = _NI, _JS, _LAG, _PF, _PPS, _U0, _UPS
    NO = JS
    S0 = S - S1
    R = M // S
    n = R // rb
    npr = rb // rr
    NP = n * npr
    nw = rb // rw
    nu = n * nw
    assert M == S * n * rb and n - JS <= NI and n - NO <= NO
    assert (LAG + PF - 1) // npr < NI and PF >= npr
    for j in range(JS):
        assert (min(NP, LAG + PF + (j + 1) * PPS) - 1) // npr - NI <= j
        assert min(NP, PF + (j + 1) * PPS) >= (j + 2) * npr
    iend = PF + JS * PPS
    uend = U0 + (n - JS) * UPS
    assert uend <= nu
    for j in range(JS, n):
        assert (U0 + (j - JS + 1) * UPS - 1) // nw <= j
        assert (j - NO + 1) * nw <= U0 + (j - JS) * UPS

    def kernel_function(x_hbm, w_hbm, o_hbm, ibuf, obuf, wbuf, rsem, wsem, ksem):
        def rd_start(p, hi):
            st = p // npr
            slot = st % NI
            q = p - st * npr
            s0, ns = (S1, S0) if hi else (0, S1)
            pltpu.make_async_copy(
                x_hbm.at[pl.ds(s0, ns), pl.ds(pl.multiple_of(p * rr, rr), rr)],
                ibuf.at[slot, pl.ds(s0, ns), pl.ds(pl.multiple_of(q * rr, rr), rr)],
                rsem.at[slot]).start(priority=0 if hi else 1)

        def rd_wait(slot):
            pltpu.make_async_copy(ibuf.at[slot], ibuf.at[slot], rsem.at[slot]).wait()

        def wr_start(u):
            st = u // nw
            slot = st % NO
            q = u - st * nw
            pltpu.make_async_copy(
                obuf.at[slot, :, pl.ds(pl.multiple_of(q * rw, rw), rw)],
                o_hbm.at[:, pl.ds(pl.multiple_of(u * rw, rw), rw)],
                wsem.at[slot]).start()

        def wr_wait(slot):
            pltpu.make_async_copy(obuf.at[slot], obuf.at[slot], wsem.at[slot]).wait()

        def compute(islot, oslot):
            xv = ibuf[islot].reshape(S * rb, C)
            y = jnp.dot(xv, wbuf[...], preferred_element_type=jnp.float32)
            obuf[oslot] = y.astype(obuf.dtype).reshape(S, rb, Co)

        def pair(i):
            @pl.when(i + LAG < NP)
            def _():
                rd_start(i + LAG, False)

            @pl.when(i < NP)
            def _():
                rd_start(i, True)

        wcp = pltpu.make_async_copy(w_hbm, wbuf, ksem)
        wcp.start()

        def lead(p, c):
            rd_start(p, False)
            return c
        jax.lax.fori_loop(0, LAG, lead, 0)

        def pairs(i, c):
            pair(i)
            return c
        jax.lax.fori_loop(0, PF, pairs, 0)
        wcp.wait()

        def phase1(j, c):
            s = j % NI
            rd_wait(s)
            compute(s, j)
            i0 = PF + j * PPS
            for q in range(PPS):
                pair(i0 + q)
            return c
        jax.lax.fori_loop(0, JS, phase1, 0)
        if iend < NP:
            jax.lax.fori_loop(iend, NP, pairs, 0)

        def drain(j, c):
            rd_wait(j % NI)
            return c
        jax.lax.fori_loop(JS, n - 1, drain, 0)

        def issue(u, c):
            wr_start(u)
            return c
        jax.lax.fori_loop(0, U0, issue, 0)
        rd_wait((n - 1) % NI)

        def phase2(j, c):
            os_ = j - NO
            wr_wait(os_)
            compute(j % NI, os_)
            u0 = U0 + (j - JS) * UPS
            for q in range(UPS):
                wr_start(u0 + q)
            return c
        jax.lax.fori_loop(JS, n, phase2, 0)

        jax.lax.fori_loop(uend, nu, issue, 0)

        def final_wait(j, c):
            wr_wait(j % NO)
            return c
        jax.lax.fori_loop(n - NO, n, final_wait, 0)

    out = pl.pallas_call(
        kernel_function,
        in_specs=[pl.BlockSpec(memory_space=pl.ANY), pl.BlockSpec(memory_space=pl.ANY)],
        out_specs=pl.BlockSpec(memory_space=pl.ANY),
        out_shape=jax.ShapeDtypeStruct((S, R, Co), x.dtype),
        scratch_shapes=[
            pltpu.VMEM((NI, S, rb, C), x.dtype),
            pltpu.VMEM((NO, S, rb, Co), x.dtype),
            pltpu.VMEM((C, Co), w.dtype),
            pltpu.SemaphoreType.DMA((NI,)),
            pltpu.SemaphoreType.DMA((NO,)),
            pltpu.SemaphoreType.DMA(()),
        ],
        compiler_params=pltpu.CompilerParams(
            vmem_limit_bytes=120 * 1024 * 1024,
            disable_bounds_checks=True,
            disable_semaphore_checks=True,
        ),
    )(x.reshape(S, R, C), w.reshape(C, Co))
    return out.reshape(B, H, W, Co)
```

```python
import jax
import jax.numpy as jnp
import jax.experimental.pallas as pl
import jax.experimental.pallas.tpu as pltpu

_S = 6
_S1 = 5
_RB = 192
_RR = 32
_RW = 48
_NI = 56
_JS = 74
_LAG = 26
_PF = 24
_PPS = 10
_KL = 4
_U0 = 64
_UPS = 6


def _compiler_params():
    vmem = 120 * 1024 * 1024
    try:
        return pltpu.CompilerParams(
            vmem_limit_bytes=vmem,
            disable_bounds_checks=True,
            disable_semaphore_checks=True,
        )
    except TypeError:
        return pltpu.CompilerParams(vmem_limit_bytes=vmem)


@jax.jit
def pallas_standalone__dilated_atrous__vision_kernel(
    x: jax.Array,
    w: jax.Array,
):
    B, H, W, C = x.shape
    Co = w.shape[-1]
    M = B * H * W
    S, S1, rb, rr, rw = _S, _S1, _RB, _RR, _RW
    NI, JS, LAG, PF, PPS, KL, U0, UPS = _NI, _JS, _LAG, _PF, _PPS, _KL, _U0, _UPS
    NO = JS
    S0 = S - S1
    R = M // S
    n = R // rb
    npr = rb // rr
    NP = n * npr
    nw = rb // rw
    nu = n * nw
    assert M == S * n * rb and n - JS <= NI and n - NO <= NO and JS < n
    assert (LAG + PF - 1) // npr < NI and PF >= npr and 0 < KL < npr
    for j in range(JS):
        assert (min(NP, LAG + PF + (j + 1) * PPS) - 1) // npr - NI <= j
        assert min(NP, PF + (j + 1) * PPS) >= (j + 2) * npr
    iend = PF + JS * PPS
    uend = U0 + (n - JS) * UPS
    assert uend <= nu
    for j in range(JS, n):
        assert (U0 + (j - JS + 1) * UPS - 1) // nw <= j
        assert (j - NO + 1) * nw <= U0 + (j - JS) * UPS

    def kernel_function(x_hbm, w_hbm, o_hbm, ibuf, obuf, wbuf, rsem, wsem, ksem):
        def rd_start(p, hi):
            st = p // npr
            slot = st % NI
            q = p - st * npr
            s0, ns = (S1, S0) if hi else (0, S1)
            sem = jnp.where(p >= NP - KL, NI, slot)
            pltpu.make_async_copy(
                x_hbm.at[pl.ds(s0, ns), pl.ds(pl.multiple_of(p * rr, rr), rr)],
                ibuf.at[slot, pl.ds(s0, ns), pl.ds(pl.multiple_of(q * rr, rr), rr)],
                rsem.at[sem]).start(priority=0 if hi else 1)

        def wait_filled(buf, sem):
            pltpu.make_async_copy(buf, buf, sem).wait()

        def wr_start(u):
            st = u // nw
            slot = st % NO
            q = u - st * nw
            pltpu.make_async_copy(
                obuf.at[slot, :, pl.ds(pl.multiple_of(q * rw, rw), rw)],
                o_hbm.at[:, pl.ds(pl.multiple_of(u * rw, rw), rw)],
                wsem.at[slot]).start()

        def wr_wait(j, slot):
            pltpu.make_async_copy(
                obuf.at[slot],
                o_hbm.at[:, pl.ds(pl.multiple_of(j * rb, rb), rb)],
                wsem.at[slot]).wait()

        def compute(islot, oslot):
            xv = ibuf[islot].reshape(S * rb, C)
            y = jnp.dot(xv, wbuf[...], preferred_element_type=jnp.float32)
            obuf[oslot] = y.astype(obuf.dtype).reshape(S, rb, Co)

        def pair(i):
            @pl.when(i + LAG < NP)
            def _():
                rd_start(i + LAG, False)

            @pl.when(i < NP)
            def _():
                rd_start(i, True)

        wcp = pltpu.make_async_copy(w_hbm, wbuf, ksem)
        wcp.start()

        def lead(p, c):
            rd_start(p, False)
            return c
        jax.lax.fori_loop(0, LAG, lead, 0)

        def pairs(i, c):
            pair(i)
            return c
        jax.lax.fori_loop(0, PF, pairs, 0)
        wcp.wait()

        def phase1(j, c):
            s = j % NI
            wait_filled(ibuf.at[s], rsem.at[s])
            compute(s, j)
            i0 = PF + j * PPS
            for q in range(PPS):
                pair(i0 + q)
            return c
        jax.lax.fori_loop(0, JS, phase1, 0)
        if iend < NP:
            jax.lax.fori_loop(iend, NP, pairs, 0)

        def drain(j, c):
            s = j % NI
            wait_filled(ibuf.at[s], rsem.at[s])
            return c
        jax.lax.fori_loop(JS, n - 1, drain, 0)
        ls = (n - 1) % NI
        cut = rb - KL * rr
        wait_filled(ibuf.at[ls, :, pl.ds(0, cut)], rsem.at[ls])

        def issue(u, c):
            wr_start(u)
            return c
        jax.lax.fori_loop(0, U0, issue, 0)
        wait_filled(ibuf.at[ls, :, pl.ds(cut, KL * rr)], rsem.at[NI])

        def phase2(j, c):
            wr_wait(j - NO, j - NO)
            compute(j % NI, j - NO)
            u0 = U0 + (j - JS) * UPS
            for q in range(UPS):
                wr_start(u0 + q)
            return c
        jax.lax.fori_loop(JS, n, phase2, 0)

        jax.lax.fori_loop(uend, nu, issue, 0)

        def final_wait(j, c):
            wr_wait(j, j % NO)
            return c
        jax.lax.fori_loop(n - NO, n, final_wait, 0)

    out = pl.pallas_call(
        kernel_function,
        in_specs=[pl.BlockSpec(memory_space=pl.ANY), pl.BlockSpec(memory_space=pl.ANY)],
        out_specs=pl.BlockSpec(memory_space=pl.ANY),
        out_shape=jax.ShapeDtypeStruct((S, R, Co), x.dtype),
        scratch_shapes=[
            pltpu.VMEM((NI, S, rb, C), x.dtype),
            pltpu.VMEM((NO, S, rb, Co), x.dtype),
            pltpu.VMEM((C, Co), w.dtype),
            pltpu.SemaphoreType.DMA((NI + 1,)),
            pltpu.SemaphoreType.DMA((NO,)),
            pltpu.SemaphoreType.DMA(()),
        ],
        compiler_params=_compiler_params(),
    )(x.reshape(S, R, C), w.reshape(C, Co))
    return out.reshape(B, H, W, Co)
```
